```python
import os as _os
_os.environ.setdefault("JAX_PLATFORMS", "cpu")
import jax
import jax.numpy as jnp

def _softmax(x, axis=-1):
    return jax.nn.softmax(x, axis=axis)
def _gelu(x):
    return jax.nn.gelu(x, approximate=True)
def _silu(x):
    return jax.nn.silu(x)
def _sigmoid(x):
    return jax.nn.sigmoid(x)
def _layernorm(x, axis=-1, eps=1e-5):
    m = jnp.mean(x, axis=axis, keepdims=True)
    v = jnp.var(x, axis=axis, keepdims=True)
    return (x - m) / jnp.sqrt(v + eps)
def _scatter_add(tgt, idx, src, axis=0):
    return tgt.at[idx].add(src)
def _segment_sum(src, seg, n):
    return jax.ops.segment_sum(src, seg, n)
class _Rng:
    def __init__(self, key):
        self._k = key
    def _next(self):
        self._k, sub = jax.random.split(self._k)
        return sub
    def normal(self, shape):
        return jax.random.normal(self._next(), shape, dtype=jnp.bfloat16)
    def randint(self, lo, hi, shape):
        return jax.random.randint(self._next(), shape, lo, hi, dtype=jnp.int32)
    def uniform(self, shape, lo=0.0, hi=1.0):
        return jax.random.uniform(self._next(), shape, jnp.bfloat16, lo, hi)
    def permutation(self, n):
        return jax.random.permutation(self._next(), n)


kernel_name = 'gated_mix__linear_kernel_hedgehog__glu_gated_bilinear__prompt'

def setup_inputs():
    _rng = _Rng(jax.random.key(int.from_bytes(__import__("os").urandom(4), "little")))
    _w = (lambda a: (lambda t: t.astype(jnp.bfloat16) if jnp.issubdtype(t.dtype, jnp.floating) else t)(jnp.asarray(a)))
    def _A_setup():
        B, S, D, H = 1, 2048, 512, 32
        Dh = D // H
        return {
            "x": _w((lambda *s: _rng.normal(s) * 0.05)(B, S, D)),
            "wqkv": _w((lambda *s: _rng.normal(s) * 0.8)(D, 3 * D)),
            "w_phi": _w((lambda *s: _rng.normal(s) * 0.8)(H, Dh, Dh) * (Dh ** -0.5)),
            "wo": _w((lambda *s: _rng.normal(s) * 0.05)(D, D)),
        }
    _A_in = _A_setup()

    def _B_setup():
        B, S, D, F = 1, 2048, 512, 1792
        return {
            "x": _w((lambda *s: _rng.normal(s) * 0.05)(B, S, D)),
            "w_gate": _w((lambda *s: _rng.normal(s) * 1.6)(D, F) * (D ** -0.5)),
            "w_up": _w((lambda *s: _rng.normal(s) * 1.6)(D, F) * (D ** -0.5)),
            "w_down": _w((lambda *s: _rng.normal(s) * 1.6)(F, D) * (F ** -0.5)),
        }
    _B_in = _B_setup()

    return {
        "A_x": _A_in["x"],
        "A_wqkv": _A_in["wqkv"],
        "A_w_phi": _A_in["w_phi"],
        "A_wo": _A_in["wo"],
        "B_x": _B_in["x"],
        "B_w_gate": _B_in["w_gate"],
        "B_w_up": _B_in["w_up"],
        "B_w_down": _B_in["w_down"],
        "gate_w": _w((lambda *s: _rng.normal(s) * 0.05)(512) * 16.0),
    }

def reference(A_x, A_wqkv, A_w_phi, A_wo, B_x, B_w_gate, B_w_up, B_w_down, gate_w):
    def _A_ref(x, wqkv, w_phi, wo):
        B, S, D = x.shape
        H = 32; Dh = D // H
        qkv = (lambda x, *d: x.transpose(*d))((x @ wqkv).reshape(B, S, 3, H, Dh), 2, 0, 3, 1, 4)
        q, k, v = qkv[0], qkv[1], qkv[2]
        pq = jnp.einsum("bhsd,hdf->bhsf", q, w_phi)
        pk = jnp.einsum("bhsd,hdf->bhsf", k, w_phi)
        phi_q = jnp.concatenate([_softmax(pq, axis=-1), _softmax(-pq, axis=-1)], axis=-1)
        phi_k = jnp.concatenate([_softmax(pk, axis=-1), _softmax(-pk, axis=-1)], axis=-1)
        kv = jnp.einsum("bhsf,bhsd->bhfd", phi_k, v)
        z  = jnp.einsum("bhsf->bhf", phi_k)
        num = jnp.einsum("bhqf,bhfd->bhqd", phi_q, kv)
        den = jnp.einsum("bhqf,bhf->bhq", phi_q, z)[..., None] + 1e-6
        o = num / den
        return (lambda x, *d: x.transpose(*d))(o, 0, 2, 1, 3).reshape(B, S, D) @ wo

    def _B_ref(x, w_gate, w_up, w_down):
        g = jnp.einsum("bsd,df->bsf", x, w_gate)
        u = jnp.einsum("bsd,df->bsf", x, w_up)
        h = g * u
        return jnp.einsum("bsf,fd->bsd", h, w_down)

    x = A_x
    g = _sigmoid((x * gate_w).sum(-1, keepdims=True))
    a = _A_ref(x, A_wqkv, A_w_phi, A_wo)
    b = _B_ref(x, B_w_gate, B_w_up, B_w_down)
    return g * a + (1 - g) * b
```

```python
import functools
import jax
import jax.numpy as jnp
import jax.experimental.pallas as pl
import jax.experimental.pallas.tpu as pltpu

_LOG2E = 1.4426950408889634
_NT = (((1,), (1,)), ((), ()))
_F32 = jnp.float32
_BF16 = jnp.bfloat16

TS = 256
FC = 256


def _iota(shape, d):
    return jax.lax.broadcasted_iota(jnp.int32, shape, d)


def _fold(w_ref, wphi_ref, dst_ref):
    r = _iota((128, 128), 0)
    c = _iota((128, 128), 1)
    mask = (r % 8) == (c // 16)
    et = (_iota((128, 16), 0) // 8 == _iota((128, 16), 1)).astype(_BF16)
    for g in range(4):
        w2 = wphi_ref[g * 128:(g + 1) * 128, :]
        pt = jax.lax.dot_general(et, w2, _NT, preferred_element_type=_F32)
        pt = jnp.where(mask, pt, 0.0).astype(_BF16)
        wt = jax.lax.dot_general(pt, w_ref[:, g * 128:(g + 1) * 128], _NT,
                                 preferred_element_type=_F32)
        dst_ref[g * 128:(g + 1) * 128, :] = (wt * _LOG2E).astype(_BF16)


def _dual_exp(p):
    rows = [p[f * 8:(f + 1) * 8, :] for f in range(16)]
    mx = functools.reduce(jnp.maximum, rows)
    mn = functools.reduce(jnp.minimum, rows)
    ep = [jnp.exp2(r - mx) for r in rows]
    en = [jnp.exp2(mn - r) for r in rows]
    sp = functools.reduce(jnp.add, ep)
    sn = functools.reduce(jnp.add, en)
    return ep, en, sp, sn


def _kernel(x_ref, wk_ref, wv_ref, wphi_ref, gw_ref, wqkv_hbm, wo_hbm, wg_hbm, wu_hbm, wd_hbm,
            o_ref,
            wq_s, wo_s, wg_s, wu_s, wd_s, wkt_s, wqt_s, kv_s, z_s, mt_s, zb_s, sems, *, n):
    i = pl.program_id(0)
    D = 512
    F = wg_s.shape[1]
    copies = [
        pltpu.make_async_copy(wqkv_hbm.at[:, pl.ds(0, D)], wq_s, sems.at[0]),
        pltpu.make_async_copy(wg_hbm, wg_s, sems.at[1]),
        pltpu.make_async_copy(wu_hbm, wu_s, sems.at[2]),
        pltpu.make_async_copy(wd_hbm, wd_s, sems.at[3]),
        pltpu.make_async_copy(wo_hbm, wo_s, sems.at[4]),
    ]

    @pl.when(i == 0)
    def _():
        for c in copies:
            c.start()
        _fold(wk_ref, wphi_ref, wkt_s)
        kv_s[...] = jnp.zeros_like(kv_s)
        z_s[...] = jnp.zeros_like(z_s)

    @pl.when(i < n)
    def _():
        x = x_ref[...]
        pk = jax.lax.dot_general(wkt_s[...], x, _NT, preferred_element_type=_F32)
        v = jnp.dot(x, wv_ref[...], preferred_element_type=_F32).astype(_BF16)
        for g in range(4):
            ep, en, sp, sn = _dual_exp(pk[g * 128:(g + 1) * 128, :])
            rp = 1.0 / sp
            rn = 1.0 / sn
            phi = jnp.concatenate([e * rp for e in ep] + [e * rn for e in en], axis=0)
            zz = phi[:, 0:128]
            for t in range(1, TS // 128):
                zz = zz + phi[:, t * 128:(t + 1) * 128]
            z_s[g] += zz
            kv_s[g] += jnp.dot(phi.astype(_BF16), v[:, g * 128:(g + 1) * 128],
                               preferred_element_type=_F32)

    @pl.when(i == n)
    def _():
        for c in copies:
            c.wait()
        _fold(wq_s, wphi_ref, wqt_s)
        r = _iota((128, 256), 0)
        c = _iota((128, 256), 1)
        mask = (r // 16) == (c % 8)
        for g in range(4):
            mt_s[g] = jnp.where(mask, kv_s[g].T, 0.0).astype(_BF16)
            zb_s[g] = jnp.broadcast_to(jnp.sum(z_s[g], axis=1, keepdims=True), (256, 128))

    @pl.when(i >= n)
    def _():
        x = x_ref[...]
        pq = jax.lax.dot_general(wqt_s[...], x, _NT, preferred_element_type=_F32)
        ots = []
        for g in range(4):
            ep, en, sp, sn = _dual_exp(pq[g * 128:(g + 1) * 128, :])
            zb = zb_s[g]
            zb = jnp.concatenate([zb] * (TS // 128), axis=1)
            tp = functools.reduce(jnp.add, [ep[f] * zb[f * 8:(f + 1) * 8] for f in range(16)])
            tn = functools.reduce(jnp.add, [en[f] * zb[128 + f * 8:128 + (f + 1) * 8] for f in range(16)])
            rp = 1.0 / sp
            rn = 1.0 / sn
            rd = 1.0 / (tp * rp + tn * rn + 1e-6)
            rp = rp * rd
            rn = rn * rd
            phi = jnp.concatenate([e * rp for e in ep] + [e * rn for e in en], axis=0)
            ots.append(jnp.dot(mt_s[g], phi.astype(_BF16), preferred_element_type=_F32))
        ot = jnp.concatenate(ots, axis=0)
        o = ot.T.astype(_BF16)
        a = jnp.dot(o, wo_s[...], preferred_element_type=_F32)
        b = None
        for c in range(F // FC):
            gg = jnp.dot(x, wg_s[:, c * FC:(c + 1) * FC], preferred_element_type=_F32)
            uu = jnp.dot(x, wu_s[:, c * FC:(c + 1) * FC], preferred_element_type=_F32)
            h = (gg * uu).astype(_BF16)
            d = jnp.dot(h, wd_s[c * FC:(c + 1) * FC, :], preferred_element_type=_F32)
            b = d if b is None else b + d
        gate = jax.nn.sigmoid(jnp.sum(x.astype(_F32) * gw_ref[...].astype(_F32), axis=1, keepdims=True))
        o_ref[...] = (gate * a + (1.0 - gate) * b).astype(o_ref.dtype)


@jax.jit
def pallas_gated_mix__linear_kernel_hedgehog__glu_gated_bilinear__prompt_kernel(
    A_x: jax.Array,
    A_wqkv: jax.Array,
    A_w_phi: jax.Array,
    A_wo: jax.Array,
    B_x: jax.Array,
    B_w_gate: jax.Array,
    B_w_up: jax.Array,
    B_w_down: jax.Array,
    gate_w: jax.Array,
):
    del B_x
    B, S, D = A_x.shape
    F = B_w_gate.shape[1]
    n = S // TS
    x = A_x.reshape(S, D)
    wphi = A_w_phi.reshape(D, A_w_phi.shape[-1])
    gw = gate_w.reshape(1, D)
    any_spec = pl.BlockSpec(memory_space=pl.ANY)
    out = pl.pallas_call(
        functools.partial(_kernel, n=n),
        grid=(2 * n,),
        in_specs=[
            pl.BlockSpec((TS, D), lambda i: (i % n, 0)),
            pl.BlockSpec((D, D), lambda i: (0, 1)),
            pl.BlockSpec((D, D), lambda i: (0, 2)),
            pl.BlockSpec(wphi.shape, lambda i: (0, 0)),
            pl.BlockSpec((1, D), lambda i: (0, 0)),
            any_spec, any_spec, any_spec, any_spec, any_spec,
        ],
        out_specs=pl.BlockSpec((TS, D), lambda i: (jnp.maximum(i - n, 0), 0)),
        out_shape=jax.ShapeDtypeStruct((S, D), A_x.dtype),
        scratch_shapes=[
            pltpu.VMEM((D, D), _BF16), pltpu.VMEM((D, D), _BF16),
            pltpu.VMEM((D, F), _BF16), pltpu.VMEM((D, F), _BF16), pltpu.VMEM((F, D), _BF16),
            pltpu.VMEM((D, D), _BF16), pltpu.VMEM((D, D), _BF16),
            pltpu.VMEM((4, 256, 128), _F32), pltpu.VMEM((4, 256, 128), _F32),
            pltpu.VMEM((4, 128, 256), _BF16), pltpu.VMEM((4, 256, 128), _F32),
            pltpu.SemaphoreType.DMA((5,)),
        ],
        compiler_params=pltpu.CompilerParams(
            dimension_semantics=("arbitrary",), vmem_limit_bytes=64 * 1024 * 1024),
    )(x, A_wqkv, A_wqkv, wphi, gw, A_wqkv, A_wo, B_w_gate, B_w_up, B_w_down)
    return out.reshape(B, S, D)
```

```python
import functools
import jax
import jax.numpy as jnp
import jax.experimental.pallas as pl
import jax.experimental.pallas.tpu as pltpu

_LOG2E = 1.4426950408889634
_NT = (((1,), (1,)), ((), ()))
_F32 = jnp.float32
_BF16 = jnp.bfloat16

T1 = 256
T2 = 512
FC = 256
U2 = False


def _iota(shape, d):
    return jax.lax.broadcasted_iota(jnp.int32, shape, d)


def _block_diag_phi(w):
    sel = (_iota((32, 512), 0) == _iota((32, 512), 1) // 16).astype(_BF16)
    a = jnp.dot(w, sel, preferred_element_type=_F32)
    a = jnp.where(_iota((256, 512), 0) // 16 == _iota((256, 512), 1) % 16, a, 0.0).astype(_BF16)
    e = (_iota((128, 256), 0) // 8 == _iota((128, 256), 1) % 16).astype(_BF16)
    pt = jnp.dot(e, a, preferred_element_type=_F32)
    keep = _iota((128, 512), 0) % 8 == (_iota((128, 512), 1) // 16) % 8
    return jnp.where(keep, pt, 0.0).astype(_BF16)


def _fold(w_ref, pt_ref, dst_ref):
    for g in range(4):
        c = slice(g * 128, (g + 1) * 128)
        wt = jax.lax.dot_general(pt_ref[:, c], w_ref[:, c], _NT, preferred_element_type=_F32)
        dst_ref[c, :] = (wt * _LOG2E).astype(_BF16)


def _dual_exp(p):
    rows = [p[f * 8:(f + 1) * 8, :] for f in range(16)]
    mx = functools.reduce(jnp.maximum, rows)
    mn = functools.reduce(jnp.minimum, rows)
    ep = [jnp.exp2(r - mx) for r in rows]
    en = [jnp.exp2(mn - r) for r in rows]
    sp = functools.reduce(jnp.add, ep)
    sn = functools.reduce(jnp.add, en)
    return ep, en, sp, sn


def _regroup(ep, en, rp, rn):
    low = _iota(rp.shape, 0) < 4
    p = [e * rp for e in ep]
    n = [pltpu.roll(e * rn, 4, 0) for e in en]
    ta = jnp.concatenate([jnp.where(low, a, b) for a, b in zip(p, n)], axis=0)
    tb = jnp.concatenate([jnp.where(low, b, a) for a, b in zip(p, n)], axis=0)
    return ta.astype(_BF16), tb.astype(_BF16)


def _kernel(wphi_hbm, gw_hbm, x_hbm, wqkv_hbm, wo_hbm, wg_hbm, wu_hbm, wd_hbm,
            o_hbm,
            wphi_ref, gw_ref, x_s, o_s, wk_s, wv_s, wq_s, wo_s, wg_s, wu_s, wd_s, pt_s, wkt_s, wqt_s, wvt_s,
            kv_s, z_s, mt_s, zb_s, sems, xsems, osems):
    S, D = x_s.shape
    F = wg_s.shape[1]
    n1, n2 = S // T1, S // T2
    cp = pltpu.make_async_copy
    x_cp = [cp(x_hbm.at[pl.ds(j * T1, T1)], x_s.at[pl.ds(j * T1, T1)], xsems.at[j]) for j in range(n1)]
    wv_cp = cp(wqkv_hbm.at[:, pl.ds(2 * D, D)], wv_s, sems.at[0])
    wk_cp = cp(wqkv_hbm.at[:, pl.ds(D, D)], wk_s, sems.at[1])
    late = [
        cp(gw_hbm, gw_ref, sems.at[8]),
        cp(wqkv_hbm.at[:, pl.ds(0, D)], wq_s, sems.at[2]),
        cp(wg_hbm, wg_s, sems.at[3]),
        cp(wu_hbm, wu_s, sems.at[4]),
        cp(wd_hbm, wd_s, sems.at[5]),
        cp(wo_hbm, wo_s, sems.at[6]),
    ]

    def o_cp(j):
        r = pl.ds(pl.multiple_of(j * T2, T2), T2)
        return cp(o_s.at[r], o_hbm.at[r], osems.at[j])

    phi_cp = cp(wphi_hbm, wphi_ref, sems.at[7])
    phi_cp.start()
    wk_cp.start()
    x_cp[0].start()
    wv_cp.start()
    phi_cp.wait()
    pt_s[...] = _block_diag_phi(wphi_ref[...])
    wk_cp.wait()
    for c in x_cp[1:]:
        c.start()
    _fold(wk_s, pt_s, wkt_s)
    x_cp[0].wait()
    wv_cp.wait()
    wvt_s[...] = wv_s[...].astype(_F32).T.astype(_BF16)

    for j in range(n1):
        if j == 1:
            for c in late:
                c.start()
            for c in x_cp[1:]:
                c.wait()
        if j == n1 - 1:
            for c in late:
                c.wait()
        x = x_s[j * T1:(j + 1) * T1, :]
        pk = jax.lax.dot_general(wkt_s[...], x, _NT, preferred_element_type=_F32)
        vt = jax.lax.dot_general(wvt_s[...], x, _NT, preferred_element_type=_F32).astype(_BF16)
        for g in range(4):
            ep, en, sp, sn = _dual_exp(pk[g * 128:(g + 1) * 128, :])
            rp = 1.0 / sp
            rn = 1.0 / sn
            phi = jnp.concatenate([e * rp for e in ep] + [e * rn for e in en], axis=0)
            zz = phi[:, 0:128]
            for t in range(1, T1 // 128):
                zz = zz + phi[:, t * 128:(t + 1) * 128]
            ta, tb = _regroup(ep, en, rp, rn)
            kv = jnp.concatenate([
                jax.lax.dot_general(vt[g * 128:g * 128 + 64], ta, _NT, preferred_element_type=_F32),
                jax.lax.dot_general(vt[g * 128 + 64:g * 128 + 128], tb, _NT, preferred_element_type=_F32),
            ], axis=0)
            if j == 0:
                z_s[g] = zz
                kv_s[g] = kv
            else:
                z_s[g] += zz
                kv_s[g] += kv

    _fold(wq_s, pt_s, wqt_s)
    mask = (_iota((128, 128), 0) // 16) % 4 == (_iota((128, 128), 1) % 4)
    for g in range(4):
        mt_s[g] = jnp.where(mask, kv_s[g], 0.0).astype(_BF16)
        zb_s[g] = jnp.broadcast_to(jnp.sum(z_s[g], axis=1, keepdims=True), (256, 128))

    def out_tile(j):
        r = pl.ds(pl.multiple_of(j * T2, T2), T2)
        x = x_s[r, :]
        pq = jax.lax.dot_general(wqt_s[...], x, _NT, preferred_element_type=_F32)
        ots = []
        for g in range(4):
            ep, en, sp, sn = _dual_exp(pq[g * 128:(g + 1) * 128, :])
            zb = zb_s[g]
            zb = jnp.concatenate([zb] * (T2 // 128), axis=1)
            tp = functools.reduce(jnp.add, [ep[f] * zb[f * 8:(f + 1) * 8] for f in range(16)])
            tn = functools.reduce(jnp.add, [en[f] * zb[128 + f * 8:128 + (f + 1) * 8] for f in range(16)])
            rp = 1.0 / sp
            rn = 1.0 / sn
            rd = 1.0 / (tp * rp + tn * rn + 1e-6)
            rp = rp * rd
            rn = rn * rd
            ta, tb = _regroup(ep, en, rp, rn)
            ots.append(jnp.dot(mt_s[g, 0:64, :], ta, preferred_element_type=_F32))
            ots.append(jnp.dot(mt_s[g, 64:128, :], tb, preferred_element_type=_F32))
        b = None
        for c in range(F // FC):
            gg = jnp.dot(x, wg_s[:, c * FC:(c + 1) * FC], preferred_element_type=_F32)
            uu = jnp.dot(x, wu_s[:, c * FC:(c + 1) * FC], preferred_element_type=_F32)
            h = (gg * uu).astype(_BF16)
            d = jnp.dot(h, wd_s[c * FC:(c + 1) * FC, :], preferred_element_type=_F32)
            b = d if b is None else b + d
        ot = jnp.concatenate(ots, axis=0)
        o = ot.T.astype(_BF16)
        a = jnp.dot(o, wo_s[...], preferred_element_type=_F32)
        gw = gw_ref[...].astype(_F32).reshape(1, D)
        gate = jax.nn.sigmoid(jnp.sum(x.astype(_F32) * gw, axis=1, keepdims=True))
        o_s[r, :] = (gate * a + (1.0 - gate) * b).astype(o_s.dtype)
        o_cp(j).start()

    if U2:
        for j in range(n2):
            out_tile(j)
    else:
        pl.loop(0, n2)(out_tile)
    for j in range(n2):
        o_cp(j).wait()


@jax.jit
def pallas_gated_mix__linear_kernel_hedgehog__glu_gated_bilinear__prompt_kernel(
    A_x: jax.Array,
    A_wqkv: jax.Array,
    A_w_phi: jax.Array,
    A_wo: jax.Array,
    B_x: jax.Array,
    B_w_gate: jax.Array,
    B_w_up: jax.Array,
    B_w_down: jax.Array,
    gate_w: jax.Array,
):
    del B_x
    B, S, D = A_x.shape
    F = B_w_gate.shape[1]
    H, Dh, _ = A_w_phi.shape
    x = A_x.reshape(S, D)
    wphi = A_w_phi.transpose(1, 2, 0).reshape(Dh * Dh, H)
    any_spec = pl.BlockSpec(memory_space=pl.ANY)
    dd = pltpu.VMEM((D, D), _BF16)
    out = pl.pallas_call(
        _kernel,
        in_specs=[any_spec] * 8,
        out_specs=any_spec,
        out_shape=jax.ShapeDtypeStruct((S, D), A_x.dtype),
        scratch_shapes=[
            pltpu.VMEM(wphi.shape, _BF16), pltpu.VMEM((D,), _BF16),
            pltpu.VMEM((S, D), _BF16), pltpu.VMEM((S, D), _BF16),
            dd, dd, dd, dd,
            pltpu.VMEM((D, F), _BF16), pltpu.VMEM((D, F), _BF16), pltpu.VMEM((F, D), _BF16),
            pltpu.VMEM((128, D), _BF16), dd, dd, dd,
            pltpu.VMEM((4, 128, 128), _F32), pltpu.VMEM((4, 256, 128), _F32),
            pltpu.VMEM((4, 128, 128), _BF16), pltpu.VMEM((4, 256, 128), _F32),
            pltpu.SemaphoreType.DMA((9,)), pltpu.SemaphoreType.DMA((S // T1,)),
            pltpu.SemaphoreType.DMA((S // T2,)),
        ],
        compiler_params=pltpu.CompilerParams(vmem_limit_bytes=96 * 1024 * 1024),
    )(wphi, gate_w, x, A_wqkv, A_wo, B_w_gate, B_w_up, B_w_down)
    return out.reshape(B, S, D)
```
